```python
import os as _os
_os.environ.setdefault("JAX_PLATFORMS", "cpu")
import jax
import jax.numpy as jnp

def _softmax(x, axis=-1):
    return jax.nn.softmax(x, axis=axis)
def _gelu(x):
    return jax.nn.gelu(x, approximate=True)
def _silu(x):
    return jax.nn.silu(x)
def _sigmoid(x):
    return jax.nn.sigmoid(x)
def _layernorm(x, axis=-1, eps=1e-5):
    m = jnp.mean(x, axis=axis, keepdims=True)
    v = jnp.var(x, axis=axis, keepdims=True)
    return (x - m) / jnp.sqrt(v + eps)
def _scatter_add(tgt, idx, src, axis=0):
    return tgt.at[idx].add(src)
def _segment_sum(src, seg, n):
    return jax.ops.segment_sum(src, seg, n)
class _Rng:
    def __init__(self, key):
        self._k = key
    def _next(self):
        self._k, sub = jax.random.split(self._k)
        return sub
    def normal(self, shape):
        return jax.random.normal(self._next(), shape, dtype=jnp.bfloat16)
    def randint(self, lo, hi, shape):
        return jax.random.randint(self._next(), shape, lo, hi, dtype=jnp.int32)
    def uniform(self, shape, lo=0.0, hi=1.0):
        return jax.random.uniform(self._next(), shape, jnp.bfloat16, lo, hi)
    def permutation(self, n):
        return jax.random.permutation(self._next(), n)


kernel_name = 'standalone__gqa_block_cached__near_ridge'

def setup_inputs():
    _rng = _Rng(jax.random.key(int.from_bytes(__import__("os").urandom(4), "little")))
    _w = (lambda a: (lambda t: t.astype(jnp.bfloat16) if jnp.issubdtype(t.dtype, jnp.floating) else t)(jnp.asarray(a)))
    B, Sq, D = 8, 80, 512
    Hq, Hkv, Sk, Dh = 32, 8, 2048, 128
    assert Hq % Hkv == 0, (Hq, Hkv)
    return {
        "x": _w((lambda *s: _rng.normal(s) * 0.8)(B, Sq, D)),
        "k_cache": _w((lambda *s: _rng.normal(s) * 0.8)(B, Hkv, Sk, Dh)),
        "v_cache": _w((lambda *s: _rng.normal(s) * 0.05)(B, Hkv, Sk, Dh)),
        "wq": _w((lambda *s: _rng.normal(s) * 0.8)(D, Hq * Dh) * (D ** -0.5)),
        "wo": _w((lambda *s: _rng.normal(s) * 0.05)(Hq * Dh, D) * ((Hq * Dh) ** -0.5)),
    }

def reference(x, k_cache, v_cache, wq, wo):
    B, Sq, D = x.shape
    Hq, Dh = 32, 128
    Hkv = k_cache.shape[1]
    rep = Hq // Hkv
    q = (lambda x, *d: x.transpose(*d))((x @ wq).reshape(B, Sq, Hq, Dh), 0, 2, 1, 3)
    k = jnp.repeat(k_cache, rep, axis=1)
    v = jnp.repeat(v_cache, rep, axis=1)
    scores = jnp.einsum("bhqd,bhkd->bhqk", q, k) * (Dh ** -0.5)
    p = _softmax(scores, axis=-1)
    o = jnp.einsum("bhqk,bhkd->bhqd", p, v)
    return (lambda x, *d: x.transpose(*d))(o, 0, 2, 1, 3).reshape(B, Sq, Hq * Dh) @ wo
```

```python
import functools
import jax, jax.numpy as jnp
from jax import lax
import jax.experimental.pallas as pl
import jax.experimental.pallas.tpu as pltpu

B, SQ, D, HQ, HKV, SK, DH = 8, 80, 512, 32, 8, 2048, 128
REP = HQ // HKV
M = REP * SQ
HD = REP * DH
LOG2E = 1.4426950408889634
NT = ((( 1,), (1,)), ((), ()))

def make(CH=512, nobc=False, dep="lrun", split=6, flags=None, fence="delay", lastdep=False, lpos=(0, 0, 1, 1), opos=2, newton=True, defer=False):
    NCH = SK // CH
    def kern(x_hbm, wq_hbm, k_hbm, v_hbm, wo_hbm, o_hbm,
             x_v, wq_v, wo_v, k_v, v_v, q_scr, a_scr, acc_scr, o_v, sem_x, sem_wq, sem_wo, sem_k, sem_v, sem_k0, sem_v0, sem_o):
        def k0_copy(b0, b1):
            return pltpu.make_async_copy(k_hbm.at[b0:b1, 0], k_v.at[0, b0:b1], sem_k0.at[b0])
        def v0_copy(b0, b1):
            return pltpu.make_async_copy(v_hbm.at[b0:b1, 0], v_v.at[0, b0:b1], sem_v0.at[b0])
        def k_copy(h):
            return pltpu.make_async_copy(k_hbm.at[:, h], k_v.at[h % 2], sem_k.at[h % 2])
        def v_copy(h):
            return pltpu.make_async_copy(v_hbm.at[:, h], v_v.at[h % 2], sem_v.at[h % 2])
        def wq_copy(h0, h1):
            return pltpu.make_async_copy(wq_hbm.at[:, h0 * HD:h1 * HD], wq_v.at[:, h0 * HD:h1 * HD], sem_wq.at[h0])
        def wo_copy(h):
            return pltpu.make_async_copy(wo_hbm.at[pl.ds(pl.multiple_of(h * HD, HD), HD), :], wo_v.at[h], sem_wo.at[h])
        x_copy = pltpu.make_async_copy(x_hbm, x_v, sem_x)

        def qk_chunk(q, slot, b, j, m_run):
            s = lax.dot_general(q, k_v[slot, b, j*CH:(j+1)*CH, :], NT, preferred_element_type=jnp.float32)
            mj = s[:, 0:128]
            for c in range(1, CH // 128):
                mj = jnp.maximum(mj, s[:, c*128:(c+1)*128])
            return s, (mj if m_run is None else jnp.maximum(m_run, mj))

        def pv_chunk(s, slot, b, j, m, l_run, acc):
            p = jnp.exp2(s - m)
            lj = p[:, 0:128]
            for c in range(1, CH // 128):
                lj = lj + p[:, c*128:(c+1)*128]
            o = jnp.dot(p.astype(jnp.bfloat16), v_v[slot, b, j*CH:(j+1)*CH, :], preferred_element_type=jnp.float32)
            return (lj if l_run is None else l_run + lj), (o if acc is None else acc + o)

        def store_o(slot, b, o):
            for r in range(REP):
                a_scr[slot, b, :, r*DH:(r+1)*DH] = o[r*SQ:(r+1)*SQ, :]

        def tie(val, tok):
            return jnp.where(tok < 0.0, tok, val)

        def tie_lhs(q, tok):
            n = q.shape[0]
            t = tok.reshape(n // 16, 2, 8, 128)
            t = jnp.minimum(t[:, 0], t[:, 1]).reshape(n // 2, 128)
            qi = pltpu.bitcast(q, jnp.int32)
            if q.shape[1] > 128:
                qi = jnp.concatenate([jnp.where(t < 0.0, 0, qi[:, :128]), qi[:, 128:]], axis=1)
            else:
                qi = jnp.where(t < 0.0, 0, qi)
            return pltpu.bitcast(qi, jnp.bfloat16)

        def step(h, b, tok, store=True):
            slot = h % 2
            m_run = None; ss = []
            for j in range(NCH):
                q = q_scr[h, b]
                if tok is not None:
                    toks = [tok[0][jj] for jj in range(NCH) if lpos[jj] == j][-1:]
                    if opos == j: toks.append(tok[1])
                    for t in toks: q = tie_lhs(q, t)
                s, m_run = qk_chunk(q, slot, b, j, m_run)
                ss.append(s)
            m = jnp.max(m_run, axis=1, keepdims=True)
            lruns = [None] * NCH
            l_run = None; acc = None
            for j in range(NCH):
                l_run, acc = pv_chunk(ss[j], slot, b, j, m, l_run, acc)
                lruns.append(l_run)
            l = jnp.sum(l_run, axis=1, keepdims=True)
            if newton:
                r0 = pl.reciprocal(l, approx=True)
                inv = r0 * (2.0 - l * r0)
            else:
                inv = 1.0 / l
            of = acc * inv
            o = of.astype(jnp.bfloat16)
            if store: store_o(slot, b, o)
            return (lruns[NCH:], jnp.abs(of)), o

        def tie_proj(a, tok, ph):
            if tok is None or not lastdep: return a
            halves = [a[:M], a[M:]]
            for i in range(2):
                j = 2 * ph + i
                toks = [tok[0][jj] for jj in range(NCH) if lpos[jj] == j][-1:]
                if opos == j: toks.append(tok[1])
                for t in toks: halves[i] = tie_lhs(halves[i], t)
            return jnp.concatenate(halves, axis=0)

        def qproj(h, rs=range(REP), tok=None):
            for i, r in enumerate(rs):
                q = jnp.dot(tie_proj(x_v[...], tok, i), wq_v[:, h*HD + r*DH:h*HD + (r+1)*DH], preferred_element_type=jnp.float32) * (DH ** -0.5 * LOG2E)
                q = q.astype(jnp.bfloat16)
                for bb in range(B):
                    q_scr[h, bb, r*SQ:(r+1)*SQ, :] = q[bb*SQ:(bb+1)*SQ, :]

        def oproj(h, mode, tok=None):
            for n in range(D // 128):
                a = tie_proj(a_scr[h % 2].reshape(B*SQ, HD), tok, n)
                y = jnp.dot(a, wo_v[h, :, n*128:(n+1)*128], preferred_element_type=jnp.float32)
                if mode == "last":
                    o_v[:, n*128:(n+1)*128] = (acc_scr[:, n*128:(n+1)*128] + y).astype(o_v.dtype)
                else:
                    acc_scr[:, n*128:(n+1)*128] += y

        x_copy.start(); wq_copy(0, 1).start()
        if fence == "delay": pl.delay(1)
        wq_copy(1, 3).start()
        acc_scr[...] = jnp.zeros_like(acc_scr)
        x_copy.wait(); wq_copy(0, 1).wait()
        wq_copy(3, HKV).start()
        qproj(0)
        wq_copy(1, 3).wait()
        k0_copy(0, split).start(); v0_copy(0, split).start()
        qproj(1); qproj(2)
        wq_copy(3, HKV).wait()
        k0_copy(split, B).start(); v0_copy(split, B).start(); wo_copy(0).start()
        for h in range(3, HKV - 1): qproj(h)
        qproj(HKV - 1, (0, 1))
        k0_copy(0, split).wait(); v0_copy(0, split).wait()
        k_copy(1).start(); v_copy(1).start(); wo_copy(1).start()
        tok = None
        for b in range(split):
            tok, o = step(0, b, tok)
        qproj(HKV - 1, (2,), tok)
        k0_copy(split, B).wait(); v0_copy(split, B).wait(); wo_copy(0).wait()
        tok = None
        for b in range(split, B):
            tok, o = step(0, b, tok)
        qproj(HKV - 1, (3,), tok)

        def head(h, _):
            wo_copy(h).wait(); k_copy(h).wait(); v_copy(h).wait()
            @pl.when(h + 1 < HKV)
            def _():
                k_copy(h + 1).start(); v_copy(h + 1).start(); wo_copy(h + 1).start()
            tok = None
            for b in range(B):
                tok, o = step(h, b, tok, store=(b < B - 1) or not defer)
            oproj(h - 1, "acc", tok)
            if defer: store_o(h % 2, B - 1, o)
        lax.fori_loop(1, HKV, head, None)
        oproj(HKV - 1, "last")
        o_copy = pltpu.make_async_copy(o_v, o_hbm, sem_o)
        o_copy.start(); o_copy.wait()

    def fn(x, k_cache, v_cache, wq, wo):
        out = pl.pallas_call(
            kern,
            in_specs=[pl.BlockSpec(memory_space=pl.ANY)] * 5,
            out_specs=pl.BlockSpec(memory_space=pl.ANY),
            out_shape=jax.ShapeDtypeStruct((B*SQ, D), jnp.bfloat16),
            scratch_shapes=[
                pltpu.VMEM((B*SQ, D), jnp.bfloat16), pltpu.VMEM((D, HQ*DH), jnp.bfloat16), pltpu.VMEM((HKV, HD, D), jnp.bfloat16),
                pltpu.VMEM((2, B, SK, DH), jnp.bfloat16), pltpu.VMEM((2, B, SK, DH), jnp.bfloat16),
                pltpu.VMEM((HKV, B, M, DH), jnp.bfloat16), pltpu.VMEM((2, B, SQ, HD), jnp.bfloat16), pltpu.VMEM((B*SQ, D), jnp.float32),
                pltpu.VMEM((B*SQ, D), jnp.bfloat16),
                pltpu.SemaphoreType.DMA(()), pltpu.SemaphoreType.DMA((HKV,)), pltpu.SemaphoreType.DMA((HKV,)),
                pltpu.SemaphoreType.DMA((2,)), pltpu.SemaphoreType.DMA((2,)),
                pltpu.SemaphoreType.DMA((B,)), pltpu.SemaphoreType.DMA((B,)), pltpu.SemaphoreType.DMA(()),
            ],
            compiler_params=pltpu.CompilerParams(vmem_limit_bytes=100*1024*1024, disable_bounds_checks=nobc, flags=flags),
        )(x.reshape(B*SQ, D), wq, k_cache, v_cache, wo)
        return out.reshape(B, SQ, D)
    return fn


_impl = make(lpos=(0, 0, 1, 1), opos=None, lastdep=True)


@jax.jit
def pallas_standalone__gqa_block_cached__near_ridge_kernel(x, k_cache, v_cache, wq, wo):
    return _impl(x, k_cache, v_cache, wq, wo)
```

```python
import jax
import jax.numpy as jnp
from jax import lax
import jax.experimental.pallas as pl
import jax.experimental.pallas.tpu as pltpu

B, SQ, D = 8, 80, 512
HQ, HKV, SK, DH = 32, 8, 2048, 128
REP = HQ // HKV
M = REP * SQ
HD = REP * DH
ROWS = B * SQ
LANES = 128
CH = 512
NCH = SK // CH
NX = 4
EARLY = 4
QSCALE = DH ** -0.5 * 1.4426950408889634
NT = (((1,), (1,)), ((), ()))

HEAD = (("P", 6, 7), ("D",), ("F",), 0, 1, ("P", 7, 8), 2, 3, ("O", 0, 2),
        4, 5, ("O", 2, 4), 6, ("O", 4, 5), 7, ("O", 5, 6))
LEFTOVER = tuple(it for it in HEAD if not isinstance(it, int) and it[0] == "P")
FIRST_HEAD = tuple(it for it in HEAD if isinstance(it, int) or it[0] == "O")

_FLAGS = ({"XLA_TPU_RESCHEDULE_DMA_DONES": True}
          if jax.__version_info__ >= (0, 12) else None)


def _order_after(lhs, tok):
    n = lhs.shape[0]
    t = tok.reshape(n // 16, 2, 8, LANES)
    t = jnp.minimum(t[:, 0], t[:, 1]).reshape(n // 2, LANES)
    bits = pltpu.bitcast(lhs, jnp.int32)
    head = jnp.where(t < 0.0, 0, bits[:, :LANES])
    if lhs.shape[1] > LANES:
        head = jnp.concatenate([head, bits[:, LANES:]], axis=1)
    return pltpu.bitcast(head, jnp.bfloat16)


def _order_rows_after(lhs, pending):
    if pending is None:
        return lhs, None
    n = min(lhs.shape[0], pending.shape[0])
    head = _order_after(lhs[:n], pending[:n])
    if n < lhs.shape[0]:
        head = jnp.concatenate([head, lhs[n:]], axis=0)
    return head, (pending[n:] if n < pending.shape[0] else None)


def _lane_tiles(a):
    return [a[:, c:c + LANES] for c in range(0, a.shape[1], LANES)]


def _kernel(x_hbm, wq_hbm, k_hbm, v_hbm, wo_hbm, o_hbm,
            x_v, wq_v, wo_v, kv_v, q_v, att_v, acc_v, o_v, l_v, u_v,
            sem_x, sem_wq0, sem_wq, sem_wo, sem_k, sem_v, sem_k0, sem_v0, sem_o):

    def rows_at(i, n):
        return pl.ds(i * n if isinstance(i, int) else pl.multiple_of(i * n, n), n)

    def x_copy(i):
        r = rows_at(i, ROWS // NX)
        return pltpu.make_async_copy(x_hbm.at[r], x_v.at[r], sem_x.at[i])

    def wq0_copy(i):
        c = rows_at(i, HD // 2)
        return pltpu.make_async_copy(wq_hbm.at[:, c], wq_v.at[0, :, c], sem_wq0.at[i])

    def wq_copy(h):
        return pltpu.make_async_copy(wq_hbm.at[:, rows_at(h, HD)], wq_v.at[h], sem_wq.at[h])

    def wo_copy(h):
        return pltpu.make_async_copy(wo_hbm.at[rows_at(h, HD)], wo_v.at[h], sem_wo.at[h])

    def k0_copy(i):
        r = pl.ds(i * (B // 2), B // 2)
        return pltpu.make_async_copy(k_hbm.at[r, 0], kv_v.at[0, 0, r], sem_k0.at[i])

    def v0_copy(i):
        r = pl.ds(i * (B // 2), B // 2)
        return pltpu.make_async_copy(v_hbm.at[r, 0], kv_v.at[0, 1, r], sem_v0.at[i])

    def k_copy(h):
        return pltpu.make_async_copy(k_hbm.at[:, h], kv_v.at[h & 1, 0], sem_k.at[h & 1])

    def v_copy(h):
        return pltpu.make_async_copy(v_hbm.at[:, h], kv_v.at[h & 1, 1], sem_v.at[h & 1])

    def o_copy(i, b0, b1):
        r = pl.ds(b0 * SQ, (b1 - b0) * SQ)
        return pltpu.make_async_copy(o_v.at[r], o_hbm.at[r], sem_o.at[i])

    def q_proj(h, heads=range(REP), b0=0, b1=B):
        for r in heads:
            q = jnp.dot(x_v[b0 * SQ:b1 * SQ, :], wq_v[h, :, r * DH:(r + 1) * DH],
                        preferred_element_type=jnp.float32)
            q = (q * QSCALE).astype(jnp.bfloat16)
            for b in range(b0, b1):
                q_v[h, b, r * SQ:(r + 1) * SQ, :] = q[(b - b0) * SQ:(b - b0 + 1) * SQ]

    def normalise(b, l_lanes, unnorm):
        l = jnp.sum(l_lanes, axis=1, keepdims=True)
        r = pl.reciprocal(l, approx=True)
        r = r * (2.0 - l * r)
        o = (unnorm * r).astype(jnp.bfloat16)
        for i in range(REP):
            att_v[b * SQ:(b + 1) * SQ, i * DH:(i + 1) * DH] = o[i * SQ:(i + 1) * SQ]

    def attention(h, b, pending, last):
        slot = h & 1
        scores, m_lanes = [], None
        for j in range(NCH):
            q, pending = _order_rows_after(q_v[h, b], pending)
            s = lax.dot_general(q, kv_v[slot, 0, b, j * CH:(j + 1) * CH, :], NT,
                                preferred_element_type=jnp.float32)
            scores.append(s)
            tiles = _lane_tiles(s)
            m = tiles[0]
            for t in tiles[1:]:
                m = jnp.maximum(m, t)
            m_lanes = m if m_lanes is None else jnp.maximum(m_lanes, m)
        m = jnp.max(m_lanes, axis=1, keepdims=True)

        sums, unnorm = [], None
        for j in range(NCH):
            p = jnp.exp2(scores[j] - m)
            tiles = _lane_tiles(p)
            l = tiles[0]
            for t in tiles[1:]:
                l = l + t
            o = jnp.dot(p.astype(jnp.bfloat16), kv_v[slot, 1, b, j * CH:(j + 1) * CH, :],
                        preferred_element_type=jnp.float32)
            sums.append(l if not sums else sums[-1] + l)
            unnorm = o if unnorm is None else unnorm + o

        if last:
            l_v[...] = sums[-1]
            u_v[...] = unnorm
            return None
        normalise(b, sums[-1], unnorm)
        return jnp.concatenate(sums, axis=0)

    def out_proj(h, b0, b1, pending, *, init=False, keep=True, emit=False):
        rows = slice(b0 * SQ, b1 * SQ)
        for c in range(0, D, LANES):
            cols = slice(c, c + LANES)
            a, pending = _order_rows_after(att_v[rows, :], pending)
            y = jnp.dot(a, wo_v[h, :, cols], preferred_element_type=jnp.float32)
            if not init:
                y = acc_v[rows, cols] + y
            if keep:
                acc_v[rows, cols] = y
            if emit:
                o_v[rows, cols] = y.astype(o_v.dtype)
        return pending

    def run_head(h, work, first):
        pending = None
        for it in work:
            if isinstance(it, int):
                if first and it == B // 2:
                    k0_copy(1).wait()
                    v0_copy(1).wait()
                pending = attention(h, it, pending, it == B - 1)
            elif it[0] == "F":
                normalise(B - 1, l_v[...], u_v[...])
            elif it[0] == "P":
                pending = out_proj(h - 1, it[1], it[2], pending)
            elif it[0] == "O":
                emit = not first and it[2] <= EARLY
                pending = out_proj(h, it[1], it[2], pending, init=first, emit=emit)
                if emit and it[2] == EARLY:
                    pl.when(h == HKV - 1)(o_copy(0, 0, EARLY).start)
            else:
                @pl.when(h + 1 < HKV)
                def _():
                    k_copy(h + 1).start()
                    v_copy(h + 1).start()
                    wo_copy(h + 1).start()

    wq0_copy(0).start()

    def start_x(i, c):
        x_copy(i).start()
        return c + i
    one = lax.fori_loop(0, NX, start_x, 1 - NX * (NX - 1) // 2)
    wq0_copy(1).start()

    def start_wq(h, c):
        wq_copy(h).start()
        return c
    lax.fori_loop(1, HKV, start_wq, 0)
    wo_copy(0).start()

    def start_kv0(i, c):
        k0_copy(i).start()
        v0_copy(i).start()
        return c
    lax.fori_loop(0, 2, start_kv0, 0)

    def prologue(_, c):
        k_copy(1).start()
        v_copy(1).start()
        wo_copy(1).start()
        for _, b0, b1 in LEFTOVER:
            acc_v[b0 * SQ:b1 * SQ, :] = jnp.zeros(((b1 - b0) * SQ, D), jnp.float32)
        wq0_copy(0).wait()
        for i in range(NX):
            x_copy(i).wait()
            q_proj(0, (0, 1), i * B // NX, (i + 1) * B // NX)
        wq0_copy(1).wait()
        q_proj(0, (2, 3))
        for h in range(1, HKV):
            wq_copy(h).wait()
            q_proj(h)
        k0_copy(0).wait()
        v0_copy(0).wait()
        wo_copy(0).wait()
        run_head(0, FIRST_HEAD, True)
        return c
    lax.fori_loop(0, one, prologue, 0)

    def head(h, c):
        wo_copy(h).wait()
        k_copy(h).wait()
        v_copy(h).wait()
        run_head(h, HEAD, False)
        return c
    lax.fori_loop(1, HKV, head, 0)

    done = min(b0 for _, b0, _ in LEFTOVER)
    o_v[EARLY * SQ:done * SQ, :] = acc_v[EARLY * SQ:done * SQ, :].astype(o_v.dtype)
    o_copy(1, EARLY, done).start()
    normalise(B - 1, l_v[...], u_v[...])
    for i, (_, b0, b1) in enumerate(LEFTOVER):
        out_proj(HKV - 1, b0, b1, None, keep=False, emit=True)
        o_copy(2 + i, b0, b1).start()
    o_copy(0, 0, EARLY).wait()
    o_copy(1, EARLY, done).wait()
    for i, (_, b0, b1) in enumerate(LEFTOVER):
        o_copy(2 + i, b0, b1).wait()


@jax.jit
def pallas_standalone__gqa_block_cached__near_ridge_kernel(
    x: jax.Array,
    k_cache: jax.Array,
    v_cache: jax.Array,
    wq: jax.Array,
    wo: jax.Array,
):
    assert x.shape == (B, SQ, D) and k_cache.shape == v_cache.shape == (B, HKV, SK, DH)
    assert wq.shape == (D, HQ * DH) and wo.shape == (HQ * DH, D)
    bf16, f32, dma = jnp.bfloat16, jnp.float32, pltpu.SemaphoreType.DMA
    out = pl.pallas_call(
        _kernel,
        in_specs=[pl.BlockSpec(memory_space=pl.ANY)] * 5,
        out_specs=pl.BlockSpec(memory_space=pl.ANY),
        out_shape=jax.ShapeDtypeStruct((ROWS, D), x.dtype),
        scratch_shapes=[
            pltpu.VMEM((ROWS, D), bf16),
            pltpu.VMEM((HKV, D, HD), bf16),
            pltpu.VMEM((HKV, HD, D), bf16),
            pltpu.VMEM((2, 2, B, SK, DH), bf16),
            pltpu.VMEM((HKV, B, M, DH), bf16),
            pltpu.VMEM((ROWS, HD), bf16),
            pltpu.VMEM((ROWS, D), f32),
            pltpu.VMEM((ROWS, D), x.dtype),
            pltpu.VMEM((M, DH), f32),
            pltpu.VMEM((M, DH), f32),
            dma((NX,)), dma((2,)), dma((HKV,)), dma((HKV,)), dma((2,)), dma((2,)),
            dma((2,)), dma((2,)), dma((2 + len(LEFTOVER),)),
        ],
        compiler_params=pltpu.CompilerParams(
            vmem_limit_bytes=64 * 1024 * 1024, flags=_FLAGS),
    )(x.reshape(ROWS, D), wq, k_cache, v_cache, wo)
    return out.reshape(B, SQ, D)
```
